```python
import jax
import jax.numpy as jnp

def _softmax(x, axis=-1):
    return jax.nn.softmax(x, axis=axis)
def _gelu(x):
    return jax.nn.gelu(x, approximate=True)
def _silu(x):
    return jax.nn.silu(x)
def _sigmoid(x):
    return jax.nn.sigmoid(x)
def _layernorm(x, axis=-1, eps=1e-5):
    m = jnp.mean(x, axis=axis, keepdims=True)
    v = jnp.var(x, axis=axis, keepdims=True)
    return (x - m) / jnp.sqrt(v + eps)
def _scatter_add(tgt, idx, src, axis=0):
    return tgt.at[idx].add(src)
def _segment_sum(src, seg, n):
    return jax.ops.segment_sum(src, seg, n)
class _Rng:
    def __init__(self, key):
        self._k = key
    def _next(self):
        self._k, sub = jax.random.split(self._k)
        return sub
    def normal(self, shape):
        return jax.random.normal(self._next(), shape, dtype=jnp.bfloat16)
    def randint(self, lo, hi, shape):
        return jax.random.randint(self._next(), shape, lo, hi, dtype=jnp.int32)
    def uniform(self, shape, lo=0.0, hi=1.0):
        return jax.random.uniform(self._next(), shape, jnp.bfloat16, lo, hi)
    def permutation(self, n):
        return jax.random.permutation(self._next(), n)


kernel_name = 'standalone__depthwise_separable__vision'

def setup_inputs():
    _rng = _Rng(jax.random.key(int.from_bytes(__import__("os").urandom(4), "little")))
    _w = (lambda a: (lambda t: t.astype(jnp.bfloat16) if jnp.issubdtype(t.dtype, jnp.floating) else t)(jnp.asarray(a)))
    H = W = 384
    C = 384
    k = 1
    return {
        "x": _w((lambda *s: _rng.normal(s) * 0.05)(1, H, W, C)),
        "dw": _w((lambda *s: _rng.normal(s) * 0.05)(k, k, C)),
        "pw": _w((lambda *s: _rng.normal(s) * 0.05)(C, C)),
    }

def reference(x, dw, pw):
    B, H, W, C = x.shape
    k = dw.shape[0]
    pad = k // 2
    xp = jnp.pad(x, ((0,0),(pad,pad),(pad,pad),(0,0)))
    out = jnp.zeros_like(x)
    for i in range(k):
        for j in range(k):
            out = out + xp[:, i:i+H, j:j+W, :] * dw[i, j][None, None, None, :]
    return jnp.einsum('bhwc,cd->bhwd', out, pw)
```

```python
import jax
import jax.numpy as jnp
from jax import lax
import jax.experimental.pallas as pl
import jax.experimental.pallas.tpu as pltpu

_STREAMS = 8
_READ_ROWS = 2304
_STEP_ROWS = 256
_WRITE_ROWS = 32


@jax.jit
def pallas_standalone__depthwise_separable__vision_kernel(
    x: jax.Array,
    dw: jax.Array,
    pw: jax.Array,
):
    B, H, W, C = x.shape
    assert dw.shape == (1, 1, C) and pw.shape == (C, C)
    S = B * H * W // _STREAMS
    assert _STREAMS * S == B * H * W and S % (2 * _READ_ROWS) == 0
    n_reads = S // _READ_ROWS
    n_steps = S // _STEP_ROWS
    steps_per_read = _READ_ROWS // _STEP_ROWS
    writes_per_step = _STEP_ROWS // _WRITE_ROWS
    half = n_steps // 2

    def kernel_function(x_hbm, dw_hbm, pw_hbm, o_hbm, buf, dw_v, pw_v,
                        read_sems, write_sem, weight_sems):
        def rows(i, n):
            return pl.ds(pl.multiple_of(i * n, n), n)

        def read(i):
            sl = rows(i, _READ_ROWS)
            return pltpu.make_async_copy(
                x_hbm.at[:, sl], buf.at[:, sl], read_sems.at[i])

        def write(j):
            sl = rows(j, _WRITE_ROWS)
            return pltpu.make_async_copy(
                buf.at[:, sl], o_hbm.at[:, sl], write_sem)

        dw_copy = pltpu.make_async_copy(dw_hbm, dw_v, weight_sems.at[0])
        pw_copy = pltpu.make_async_copy(pw_hbm, pw_v, weight_sems.at[1])
        dw_copy.start()
        pw_copy.start()
        lax.fori_loop(0, n_reads, lambda i, _: read(i).start(), None)
        dw_copy.wait()
        pw_copy.wait()
        scale = dw_v[0].astype(jnp.float32)

        def compute(t):
            sl = rows(t, _STEP_ROWS)
            xv = buf[:, sl, :].reshape(_STREAMS * _STEP_ROWS, C)
            y = (xv.astype(jnp.float32) * scale).astype(buf.dtype)
            o = jnp.dot(y, pw_v[...], preferred_element_type=jnp.float32)
            buf[:, sl, :] = o.astype(buf.dtype).reshape(_STREAMS, _STEP_ROWS, C)

        def first_half(t, _):
            @pl.when(t % steps_per_read == 0)
            def _():
                read(t // steps_per_read).wait()

            compute(t)

        lax.fori_loop(0, half, first_half, None)
        for i in range(n_reads // 2, n_reads):
            read(i).wait()

        def second_half(u, _):
            for q in range(2 * writes_per_step):
                write(u * 2 * writes_per_step + q).start()
            compute(half + u)

        lax.fori_loop(0, half - 1, second_half, None)
        compute(n_steps - 1)
        for q in range(2 * writes_per_step):
            write((half - 1) * 2 * writes_per_step + q).start()
        pltpu.make_async_copy(buf, o_hbm, write_sem).wait()

    out = pl.pallas_call(
        kernel_function,
        in_specs=[pl.BlockSpec(memory_space=pl.ANY)] * 3,
        out_specs=pl.BlockSpec(memory_space=pl.ANY),
        out_shape=jax.ShapeDtypeStruct((_STREAMS, S, C), x.dtype),
        scratch_shapes=[
            pltpu.VMEM((_STREAMS, S, C), x.dtype),
            pltpu.VMEM(dw.shape, dw.dtype),
            pltpu.VMEM(pw.shape, pw.dtype),
            pltpu.SemaphoreType.DMA((n_reads,)),
            pltpu.SemaphoreType.DMA(()),
            pltpu.SemaphoreType.DMA((2,)),
        ],
        compiler_params=pltpu.CompilerParams(vmem_limit_bytes=126 * 2**20),
    )(x.reshape(_STREAMS, S, C), dw, pw)
    return out.reshape(B, H, W, C)
```

```python
import jax
import jax.numpy as jnp
from jax import lax
import jax.experimental.pallas as pl
import jax.experimental.pallas.tpu as pltpu

_STREAMS = 6
_STEP_ROWS = 192
_READ_ROWS = 32
_WRITE_ROWS = 48
_READ_AHEAD = 6
_TAIL_READS = 6
_FIRST_WRITES = 4


@jax.jit
def pallas_standalone__depthwise_separable__vision_kernel(
    x: jax.Array,
    dw: jax.Array,
    pw: jax.Array,
):
    B, H, W, C = x.shape
    assert dw.shape == (1, 1, C) and pw.shape == (C, C)
    S = B * H * W // _STREAMS
    group_rows = 2 * _STEP_ROWS
    assert _STREAMS * S == B * H * W and S % group_rows == 0
    n_steps = S // _STEP_ROWS
    n_groups = S // group_rows
    reads_per_group = group_rows // _READ_ROWS
    writes_per_step = _STEP_ROWS // _WRITE_ROWS
    n_sems = _READ_AHEAD + 1
    turn = n_groups - _READ_AHEAD + 1
    assert _FIRST_WRITES <= turn < n_groups

    def kernel_function(x_hbm, dw_hbm, pw_hbm, o_hbm, buf, dw_v, pw_v,
                        read_sems, tail_sem, write_sem):
        def rows(i, n, size=None):
            return pl.ds(pl.multiple_of(i * n, n), size or n)

        def start_reads(lo, hi, sem):
            def start_pair(i, _):
                for p in range(2):
                    streams = pl.ds(p * (_STREAMS // 2), _STREAMS // 2)
                    sl = rows(i, _READ_ROWS)
                    pltpu.make_async_copy(
                        x_hbm.at[streams, sl], buf.at[streams, sl], sem
                    ).start(priority=p)

            lax.fori_loop(lo, hi, start_pair, None)

        def wait_reads(sl, sem):
            pltpu.make_async_copy(x_hbm.at[:, sl], buf.at[:, sl], sem).wait()

        def group_sem(g):
            return read_sems.at[lax.rem(g, n_sems)]

        def start_group(g):
            start_reads(g * reads_per_group, (g + 1) * reads_per_group,
                        group_sem(g))

        def start_writes(lo, hi):
            def start_one(i, _):
                sl = rows(i, _WRITE_ROWS)
                pltpu.make_async_copy(
                    buf.at[:, sl], o_hbm.at[:, sl], write_sem).start()

            lax.fori_loop(lo * writes_per_step, hi * writes_per_step,
                          start_one, None)

        dw_copy = pltpu.make_async_copy(dw_hbm, dw_v, write_sem)
        pw_copy = pltpu.make_async_copy(pw_hbm, pw_v, write_sem)
        dw_copy.start()
        pw_copy.start()
        lax.fori_loop(0, _READ_AHEAD, lambda g, _: start_group(g), None)
        dw_copy.wait()
        pw_copy.wait()
        scale = dw_v[0].astype(jnp.float32)

        last = n_groups - 1
        n_reads = n_groups * reads_per_group
        tail_rows = _TAIL_READS * _READ_ROWS

        def step(t, _):
            @pl.when(t + _READ_AHEAD < last)
            def _():
                start_group(t + _READ_AHEAD)

            @pl.when(t + _READ_AHEAD == last)
            def _():
                start_reads(last * reads_per_group, n_reads - _TAIL_READS,
                            group_sem(last))
                start_reads(n_reads - _TAIL_READS, n_reads, tail_sem)

            @pl.when(t < turn)
            def _():
                wait_reads(rows(t, group_rows), group_sem(t))

            @pl.when(t == turn)
            def _():
                for g in range(turn, last):
                    wait_reads(rows(g, group_rows), group_sem(g))
                wait_reads(rows(last, group_rows, group_rows - tail_rows),
                           group_sem(last))
                start_writes(0, _FIRST_WRITES)
                wait_reads(pl.ds(S - tail_rows, tail_rows), tail_sem)

            @pl.when(t > turn)
            def _():
                start_writes(
                    jnp.minimum(t - 1, _FIRST_WRITES + 2 * (t - 1 - turn)),
                    jnp.minimum(t, _FIRST_WRITES + 2 * (t - turn)))

            sl = rows(t, _STEP_ROWS)
            xv = buf[:, sl, :].reshape(_STREAMS * _STEP_ROWS, C)
            y = (xv.astype(jnp.float32) * scale).astype(buf.dtype)
            o = jnp.dot(y, pw_v[...], preferred_element_type=jnp.float32)
            buf[:, sl, :] = o.astype(buf.dtype).reshape(_STREAMS, _STEP_ROWS, C)

        lax.fori_loop(0, n_steps, step, None)
        start_writes(
            min(n_steps - 1, _FIRST_WRITES + 2 * (n_steps - 1 - turn)), n_steps)
        pltpu.make_async_copy(buf, o_hbm, write_sem).wait()

    out = pl.pallas_call(
        kernel_function,
        in_specs=[pl.BlockSpec(memory_space=pl.ANY)] * 3,
        out_specs=pl.BlockSpec(memory_space=pl.ANY),
        out_shape=jax.ShapeDtypeStruct((_STREAMS, S, C), x.dtype),
        scratch_shapes=[
            pltpu.VMEM((_STREAMS, S, C), x.dtype),
            pltpu.VMEM(dw.shape, dw.dtype),
            pltpu.VMEM(pw.shape, pw.dtype),
            pltpu.SemaphoreType.DMA((n_sems,)),
            pltpu.SemaphoreType.DMA(()),
            pltpu.SemaphoreType.DMA(()),
        ],
        compiler_params=pltpu.CompilerParams(vmem_limit_bytes=126 * 2**20),
    )(x.reshape(_STREAMS, S, C), dw, pw)
    return out.reshape(B, H, W, C)
```

```python
import jax
import jax.numpy as jnp
from jax import lax
import jax.experimental.pallas as pl
import jax.experimental.pallas.tpu as pltpu

_STREAMS = 6
_STEP_ROWS = 192
_READ_ROWS = 32
_WRITE_ROWS = 48
_READ_AHEAD = 6
_TAIL_READS = 7
_FIRST_WRITES = 4


@jax.jit
def pallas_standalone__depthwise_separable__vision_kernel(
    x: jax.Array,
    dw: jax.Array,
    pw: jax.Array,
):
    B, H, W, C = x.shape
    assert dw.shape == (1, 1, C) and pw.shape == (C, C)
    S = B * H * W // _STREAMS
    group_rows = 2 * _STEP_ROWS
    assert _STREAMS * S == B * H * W and S % group_rows == 0
    n_steps = S // _STEP_ROWS
    n_groups = S // group_rows
    reads_per_group = group_rows // _READ_ROWS
    writes_per_step = _STEP_ROWS // _WRITE_ROWS
    n_sems = _READ_AHEAD + 1
    turn = n_groups - _READ_AHEAD + 1
    assert _FIRST_WRITES <= turn < n_groups

    def kernel_function(x_hbm, dw_hbm, pw_hbm, o_hbm, buf, dw_v, pw_v,
                        read_sems, tail_sem, write_sem):
        def rows(i, n, size=None):
            return pl.ds(pl.multiple_of(i * n, n), size or n)

        def start_reads(lo, hi, sem, priorities=(0, 1)):
            def start_pair(i, _):
                for half, priority in enumerate(priorities):
                    streams = pl.ds(half * (_STREAMS // 2), _STREAMS // 2)
                    sl = rows(i, _READ_ROWS)
                    pltpu.make_async_copy(
                        x_hbm.at[streams, sl], buf.at[streams, sl], sem
                    ).start(priority=priority)

            lax.fori_loop(lo, hi, start_pair, None)

        def wait_reads(sl, sem):
            pltpu.make_async_copy(x_hbm.at[:, sl], buf.at[:, sl], sem).wait()

        def group_sem(g):
            return read_sems.at[lax.rem(g, n_sems)]

        def start_group(g):
            start_reads(g * reads_per_group, (g + 1) * reads_per_group,
                        group_sem(g))

        def start_writes(lo, hi):
            def start_one(i, _):
                sl = rows(i, _WRITE_ROWS)
                pltpu.make_async_copy(
                    buf.at[:, sl], o_hbm.at[:, sl], write_sem).start()

            lax.fori_loop(lo * writes_per_step, hi * writes_per_step,
                          start_one, None)

        dw_copy = pltpu.make_async_copy(dw_hbm, dw_v, write_sem)
        pw_copy = pltpu.make_async_copy(pw_hbm, pw_v, write_sem)
        dw_copy.start()
        pw_copy.start()
        start_reads(0, reads_per_group, read_sems.at[0], priorities=(1, 1))
        lax.fori_loop(1, _READ_AHEAD, lambda g, _: start_group(g), None)
        dw_copy.wait()
        pw_copy.wait()
        scale = dw_v[0].astype(jnp.float32)

        last = n_groups - 1
        n_reads = n_groups * reads_per_group
        tail_rows = _TAIL_READS * _READ_ROWS

        def step(t, _):
            @pl.when(t + _READ_AHEAD < last)
            def _():
                start_group(t + _READ_AHEAD)

            @pl.when(t + _READ_AHEAD == last)
            def _():
                start_reads(last * reads_per_group, n_reads - _TAIL_READS,
                            group_sem(last))
                start_reads(n_reads - _TAIL_READS, n_reads, tail_sem)

            @pl.when(t < turn)
            def _():
                wait_reads(rows(t, group_rows), group_sem(t))

            @pl.when(t == turn)
            def _():
                for g in range(turn, last):
                    wait_reads(rows(g, group_rows), group_sem(g))
                wait_reads(rows(last, group_rows, group_rows - tail_rows),
                           group_sem(last))
                start_writes(0, _FIRST_WRITES)
                wait_reads(pl.ds(S - tail_rows, tail_rows), tail_sem)

            @pl.when(t > turn)
            def _():
                start_writes(
                    jnp.minimum(t - 1, _FIRST_WRITES + 2 * (t - 1 - turn)),
                    jnp.minimum(t, _FIRST_WRITES + 2 * (t - turn)))

            sl = rows(t, _STEP_ROWS)
            xv = buf[:, sl, :].reshape(_STREAMS * _STEP_ROWS, C)
            y = (xv.astype(jnp.float32) * scale).astype(buf.dtype)
            o = jnp.dot(y, pw_v[...], preferred_element_type=jnp.float32)
            buf[:, sl, :] = o.astype(buf.dtype).reshape(_STREAMS, _STEP_ROWS, C)

        lax.fori_loop(0, n_steps, step, None)
        start_writes(
            min(n_steps - 1, _FIRST_WRITES + 2 * (n_steps - 1 - turn)), n_steps)
        pltpu.make_async_copy(buf, o_hbm, write_sem).wait()

    out = pl.pallas_call(
        kernel_function,
        in_specs=[pl.BlockSpec(memory_space=pl.ANY)] * 3,
        out_specs=pl.BlockSpec(memory_space=pl.ANY),
        out_shape=jax.ShapeDtypeStruct((_STREAMS, S, C), x.dtype),
        scratch_shapes=[
            pltpu.VMEM((_STREAMS, S, C), x.dtype),
            pltpu.VMEM(dw.shape, dw.dtype),
            pltpu.VMEM(pw.shape, pw.dtype),
            pltpu.SemaphoreType.DMA((n_sems,)),
            pltpu.SemaphoreType.DMA(()),
            pltpu.SemaphoreType.DMA(()),
        ],
        compiler_params=pltpu.CompilerParams(vmem_limit_bytes=116 * 2**20),
    )(x.reshape(_STREAMS, S, C), dw, pw)
    return out.reshape(B, H, W, C)
```
